```python
import os as _os
_os.environ.setdefault("JAX_PLATFORMS", "cpu")
import jax
import jax.numpy as jnp

def _softmax(x, axis=-1):
    return jax.nn.softmax(x, axis=axis)
def _gelu(x):
    return jax.nn.gelu(x, approximate=True)
def _silu(x):
    return jax.nn.silu(x)
def _sigmoid(x):
    return jax.nn.sigmoid(x)
def _layernorm(x, axis=-1, eps=1e-5):
    m = jnp.mean(x, axis=axis, keepdims=True)
    v = jnp.var(x, axis=axis, keepdims=True)
    return (x - m) / jnp.sqrt(v + eps)
def _scatter_add(tgt, idx, src, axis=0):
    return tgt.at[idx].add(src)
def _segment_sum(src, seg, n):
    return jax.ops.segment_sum(src, seg, n)
class _Rng:
    def __init__(self, key):
        self._k = key
    def _next(self):
        self._k, sub = jax.random.split(self._k)
        return sub
    def normal(self, shape):
        return jax.random.normal(self._next(), shape, dtype=jnp.bfloat16)
    def randint(self, lo, hi, shape):
        return jax.random.randint(self._next(), shape, lo, hi, dtype=jnp.int32)
    def uniform(self, shape, lo=0.0, hi=1.0):
        return jax.random.uniform(self._next(), shape, jnp.bfloat16, lo, hi)
    def permutation(self, n):
        return jax.random.permutation(self._next(), n)


kernel_name = 'interleave_layers__linear_attn_block__mha_block__prompt'

def setup_inputs():
    _rng = _Rng(jax.random.key(int.from_bytes(__import__("os").urandom(4), "little")))
    _w = (lambda a: (lambda t: t.astype(jnp.bfloat16) if jnp.issubdtype(t.dtype, jnp.floating) else t)(jnp.asarray(a)))
    def _A_setup():
        B, S, D = 1, 2048, 640
        return {
            "x": _w((lambda *s: _rng.normal(s) * 0.05)(B, S, D)),
            "wqkv": _w((lambda *s: _rng.normal(s) * 0.1)(D, 3 * D)),
            "wo": _w((lambda *s: _rng.normal(s) * 0.05)(D, D)),
        }
    _A_in = _A_setup()

    def _B_setup():
        B, S, D, H = 1, 2048, 640, 32
        return {
            "x": _w((lambda *s: _rng.normal(s) * 0.05)(B, S, D)),
            "wqkv": _w((lambda *s: _rng.normal(s) * 0.1)(D, 3 * D)),
            "wo": _w((lambda *s: _rng.normal(s) * 0.05)(D, D)),
        }
    _B_in = _B_setup()

    return {
        "A_x": _A_in["x"],
        "A_wqkv": _A_in["wqkv"],
        "A_wo": _A_in["wo"],
        "B_x": _B_in["x"],
        "B_wqkv": _B_in["wqkv"],
        "B_wo": _B_in["wo"],
    }

def reference(A_x, A_wqkv, A_wo, B_x, B_wqkv, B_wo):
    def _A_ref(x, wqkv, wo):
        B, S, D = x.shape
        H = 32; Dh = D // H
        qkv = (lambda x, *d: x.transpose(*d))((x @ wqkv).reshape(B, S, 3, H, Dh), 2, 0, 3, 1, 4)
        q, k, v = qkv[0], qkv[1], qkv[2]
        phi = lambda t: jnp.where(t > 0, t + 1, jnp.exp(t)) + 1e-6
        pq, pk = phi(q), phi(k)
        kv = jnp.einsum("bhsd,bhse->bhde", pk, v)
        z = jnp.einsum("bhsd->bhd", pk)
        num = jnp.einsum("bhqd,bhde->bhqe", pq, kv)
        den = jnp.einsum("bhqd,bhd->bhq", pq, z)[..., None] + 1e-6
        o = num / den
        return (lambda x, *d: x.transpose(*d))(o, 0, 2, 1, 3).reshape(B, S, D) @ wo

    def _B_ref(x, wqkv, wo):
        B, S, D = x.shape
        H = 32
        Dh = D // H
        qkv = (lambda x, *d: x.transpose(*d))((x @ wqkv).reshape(B, S, 3, H, Dh), 2, 0, 3, 1, 4)
        q, k, v = qkv[0], qkv[1], qkv[2]
        scores = jnp.einsum("bhqd,bhkd->bhqk", q, k) * (Dh ** -0.5)
        p = _softmax(scores, axis=-1)
        o = jnp.einsum("bhqk,bhkd->bhqd", p, v)
        return (lambda x, *d: x.transpose(*d))(o, 0, 2, 1, 3).reshape(B, S, D) @ wo

    x = A_x
    x = x + _A_ref(_layernorm(x, axis=-1), A_wqkv, A_wo)
    x = x + _B_ref(_layernorm(x, axis=-1), B_wqkv, B_wo)
    x = x + _A_ref(_layernorm(x, axis=-1), A_wqkv, A_wo)
    x = x + _B_ref(_layernorm(x, axis=-1), B_wqkv, B_wo)
    return x
```

```python
import functools
import math

import jax
import jax.numpy as jnp
from jax import lax
import jax.experimental.pallas as pl
import jax.experimental.pallas.tpu as pltpu

S = 2048
D = 640
H = 32
DH = D // H
WIN = 128
WIN_START = (0, 120, 240, 360, 480, 512)
TC = 512
QB = 512
KC = 128
NQ = S // QB
F32 = jnp.float32
BF16 = jnp.bfloat16

_NT = (((1,), (1,)), ((), ()))


def _mm(a, b):
    return jnp.dot(a, b, preferred_element_type=F32)


def _phi(t):
    return jnp.where(t > 0, t + 1.0, jnp.exp(t)) + 1e-6


def _kernel(x_ref, waq_ref, wao_ref, wbq_ref, wbo_ref, o_ref,
            xt, xn, waq_t, wao_t, wbq_t, wbo_t, qt, vt, ot, wq, wk, wv, kw, s0, s1):

    def tok(c, n=TC):
        return pl.ds(pl.multiple_of(c * n, n), n)

    def load_x(c, _):
        xt[:, tok(c)] = x_ref[tok(c), :].astype(F32).T
        return 0
    lax.fori_loop(0, S // TC, load_x, 0)
    for src, dst in ((waq_ref, waq_t), (wao_ref, wao_t), (wbq_ref, wbq_t), (wbo_ref, wbo_t)):
        for j in range(src.shape[1] // D):
            dst[j * D:(j + 1) * D, :] = src[:, j * D:(j + 1) * D].astype(F32).T.astype(BF16)

    def layernorm(c):
        x = xt[:, tok(c)]
        m = jnp.mean(x, axis=0, keepdims=True)
        xc = x - m
        v = jnp.mean(xc * xc, axis=0, keepdims=True)
        return (xc / jnp.sqrt(v + 1e-5)).astype(BF16)

    def out_proj(w_t):
        def body(c, _):
            xt[:, tok(c)] += _mm(w_t[...], ot[:, tok(c)].astype(BF16))
            return 0
        lax.fori_loop(0, S // TC, body, 0)

    def linear_attn_layer():
        def proj(c, _):
            n = layernorm(c)
            for j, (dst, fn) in enumerate(((wq, _phi), (wk, _phi), (wv, None))):
                y = _mm(waq_t[j * D:(j + 1) * D, :], n)
                if fn is not None:
                    y = fn(y)
                for w, r0 in enumerate(WIN_START):
                    yw = y[r0:r0 + WIN]
                    if fn is None:
                        row = lax.broadcasted_iota(jnp.int32, yw.shape, 0)
                        yw = jnp.where(row < 8 if w == 5 else row >= 120, 1.0, yw)
                    dst[w, :, tok(c)] = yw.astype(BF16)
            return 0
        lax.fori_loop(0, S // TC, proj, 0)

        for w, r0 in enumerate(WIN_START):
            kvz = lax.dot_general(wv[w], wk[w], _NT, preferred_element_type=F32)
            e = lax.broadcasted_iota(jnp.int32, kvz.shape, 0)
            d = lax.broadcasted_iota(jnp.int32, kvz.shape, 1)
            if w == 5:
                heads, first, zrow = (30, 31), 88, 0
            else:
                heads, first, zrow = tuple(range(6 * w, 6 * w + 6)), 0, 120
            keep = None
            for j in range(len(heads)):
                lo = first + j * DH
                in_d = (d >= lo) & (d < lo + DH)
                in_e = ((e >= lo) & (e < lo + DH)) | (e == zrow + j)
                blk = in_d & in_e
                keep = blk if keep is None else keep | blk
            kvz = jnp.where(keep, kvz, 0.0).astype(BF16)

            def apply(c, _, w=w, r0=r0, kvz=kvz, heads=heads, first=first, zrow=zrow):
                nd = _mm(kvz, wq[w, :, tok(c)])
                den = nd[zrow:zrow + 8] + 1e-6
                for g in range(len(heads) * DH // 8):
                    a = first + 8 * g
                    j0, j1 = (8 * g) // DH, (8 * g + 7) // DH
                    dg = jnp.broadcast_to(den[j0:j0 + 1], (8, TC))
                    if j1 != j0:
                        row = lax.broadcasted_iota(jnp.int32, (8, TC), 0)
                        dg = jnp.where(row < j1 * DH - 8 * g, dg,
                                       jnp.broadcast_to(den[j1:j1 + 1], (8, TC)))
                    ot[r0 + a:r0 + a + 8, tok(c)] = nd[a:a + 8] / dg
                return 0
            lax.fori_loop(0, S // TC, apply, 0)
        out_proj(wao_t)

    def mha_layer():
        def proj(c, _):
            n = layernorm(c)
            qt[:, tok(c)] = _mm(wbq_t[0:D, :], n) * (DH ** -0.5 * math.log2(math.e))
            k = _mm(wbq_t[D:2 * D, :], n)
            for w, r0 in enumerate(WIN_START):
                kw[w, tok(c), :] = k[r0:r0 + WIN].T.astype(BF16)
            vt[:, tok(c)] = _mm(wbq_t[2 * D:3 * D, :], n)
            return 0
        lax.fori_loop(0, S // TC, proj, 0)

        def stage(new, s_new, old, s_old, m_old):
            if new is not None:
                pair, qb, par = new
                w = jnp.minimum(pair // 3, 5)
                r0 = pl.multiple_of(jnp.minimum(w * 120, 512), 8)
                q = qt[pl.ds(r0, WIN), tok(qb, QB)]
                row = lax.broadcasted_iota(jnp.int32, q.shape, 0) + r0
                lo = pair * (2 * DH) + par * DH
                qm = jnp.where((row >= lo) & (row < lo + DH), q, 0.0).astype(BF16)
                mx = None
            if old is not None:
                pair_o, _, par_o = old
                v0 = pl.multiple_of(pair_o * (2 * DH) + 16 * par_o, 8)
                vrow = lax.broadcasted_iota(jnp.int32, (24, KC), 0)
                ones = vrow < 4 if par_o else vrow >= DH
                acc = None
            for j in range(S // KC):
                ks = slice(j * KC, (j + 1) * KC)
                if new is not None:
                    s = _mm(kw[w, ks, :], qm)
                    s_new[ks, :] = s
                    cm = jnp.max(s.reshape(KC // 8, 8, QB), axis=0)
                    mx = cm if mx is None else jnp.maximum(mx, cm)
                if old is not None:
                    p = jnp.exp2(s_old[ks, :] - m_old)
                    pv = _mm(jnp.where(ones, 1.0, vt[pl.ds(v0, 24), ks]), p)
                    acc = pv if acc is None else acc + pv
            o = m = None
            if old is not None:
                l = acc[0:1] if par_o else acc[DH:DH + 1]
                o = acc / l
            if new is not None:
                m = jnp.max(mx, axis=0, keepdims=True)
            return o, m

        n_items = (H // 2) * NQ
        _, m0 = stage((0, 0, 0), s0, None, None, None)

        def body(t, m):
            pair, qb = t // NQ, t % NQ
            tn = jnp.minimum(t + 1, n_items - 1)
            o_e, m = stage((pair, qb, 1), s1, (pair, qb, 0), s0, m)
            o_o, m = stage((tn // NQ, tn % NQ, 0), s0, (pair, qb, 1), s1, m)
            row = lax.broadcasted_iota(jnp.int32, (8, QB), 0)
            a = pl.multiple_of(pair * (2 * DH), 8)
            ot[pl.ds(a, 16), tok(qb, QB)] = o_e[0:16]
            ot[pl.ds(a + 16, 8), tok(qb, QB)] = jnp.where(row < 4, o_e[16:24], o_o[0:8])
            ot[pl.ds(a + 24, 16), tok(qb, QB)] = o_o[8:24]
            return m
        lax.fori_loop(0, n_items, body, m0)
        out_proj(wbo_t)

    def layer_pair(_, c):
        linear_attn_layer()
        mha_layer()
        return c
    lax.fori_loop(0, 2, layer_pair, 0)

    def store(c, _):
        o_ref[tok(c), :] = xt[:, tok(c)].T.astype(o_ref.dtype)
        return 0
    lax.fori_loop(0, S // TC, store, 0)


@jax.jit
def pallas_interleave_layers__linear_attn_block__mha_block__prompt_kernel(
    A_x: jax.Array,
    A_wqkv: jax.Array,
    A_wo: jax.Array,
    B_x: jax.Array,
    B_wqkv: jax.Array,
    B_wo: jax.Array,
):
    del B_x
    vmem = pltpu.VMEM
    out = pl.pallas_call(
        _kernel,
        out_shape=jax.ShapeDtypeStruct((S, D), A_x.dtype),
        scratch_shapes=[
            vmem((D, S), F32),
            vmem((D, S), BF16),
            vmem((3 * D, D), BF16), vmem((D, D), BF16),
            vmem((3 * D, D), BF16), vmem((D, D), BF16),
            vmem((D, S), F32), vmem((D, S), F32), vmem((D, S), F32),
            vmem((6, WIN, S), BF16), vmem((6, WIN, S), BF16), vmem((6, WIN, S), BF16),
            vmem((6, S, WIN), BF16),
            vmem((S, QB), F32), vmem((S, QB), F32),
        ],
        compiler_params=pltpu.CompilerParams(vmem_limit_bytes=100 * 1024 * 1024),
        name="interleaved_attn",
    )(A_x.reshape(S, D), A_wqkv, A_wo, B_wqkv, B_wo)
    return out.reshape(A_x.shape)
```

```python
import math

import jax
import jax.numpy as jnp
from jax import lax
import jax.experimental.pallas as pl
import jax.experimental.pallas.tpu as pltpu

S = 2048
D = 640
H = 32
DH = D // H
PW = 2 * DH
WIN = 128
WIN_START = (0, 120, 240, 360, 480, 592)
TC = 512
NT = S // TC
QB = 512
NQ = S // QB
KC = 128
NCH = S // KC
LAG = 3
UNROLL = 3
F32 = jnp.float32
BF16 = jnp.bfloat16

_NT = (((1,), (1,)), ((), ()))


def _mm(a, b):
    return jnp.dot(a, b, preferred_element_type=F32)


def _phi(t):
    return jnp.where(t > 0, t + 1.0, jnp.exp(t)) + 1e-6


def _layernorm(x):
    m = jnp.mean(x, axis=0, keepdims=True)
    xc = x - m
    v = jnp.mean(xc * xc, axis=0, keepdims=True)
    return (xc / jnp.sqrt(v + 1e-5)).astype(BF16)


def _win_layout(w):
    return (48, 2, 8, 0) if w == 5 else (WIN, 6, 0, 120)


def _kernel(x_hbm, waq_hbm, wao_hbm, wbq_hbm, wbo_hbm, o_hbm,
            xio, wst, wt_a, wt_r, xt, xn, pq, kv, kvz, qt, kw, vt, ot, s0, s1,
            x_sem, w_sem, o_sem):

    def tok(c):
        return pl.ds(pl.multiple_of(c * TC, TC), TC)

    def x_copy(c):
        return pltpu.make_async_copy(x_hbm.at[tok(c), :], xio.at[tok(c), :], x_sem.at[c])

    def o_copy(c):
        return pltpu.make_async_copy(xio.at[tok(c), :], o_hbm.at[tok(c), :], o_sem.at[c])

    w_src = ([waq_hbm.at[:, j * D:(j + 1) * D] for j in range(3)] + [wao_hbm]
             + [wbq_hbm.at[:, j * D:(j + 1) * D] for j in range(3)] + [wbo_hbm])
    w_copies = [pltpu.make_async_copy(src, wst.at[:, j * D:(j + 1) * D], w_sem.at[j])
                for j, src in enumerate(w_src)]

    def transpose_weights(dst, base, start, size):
        start = pl.multiple_of(start, 128)
        cols = pl.ds(pl.multiple_of(base + start, 128), size)
        dst[pl.ds(start, size), :] = wst[:, cols].astype(F32).T.astype(BF16)

    def a_proj(c, n):
        q = _phi(_mm(wt_a[0:D, :], n))
        k = _phi(_mm(wt_a[D:2 * D, :], n))
        v = _mm(wt_a[2 * D:3 * D, :], n)
        for w, r0 in enumerate(WIN_START):
            n_r, _, _, spare = _win_layout(w)
            pq[w, :n_r, tok(c)] = q[r0:r0 + n_r].astype(BF16)
            row = lax.broadcasted_iota(jnp.int32, (n_r, TC), 0)
            vw = jnp.where((row >= spare) & (row < spare + 8), 1.0, v[r0:r0 + n_r])
            kv[w, :n_r, :n_r] += lax.dot_general(
                vw.astype(BF16), k[r0:r0 + n_r].astype(BF16), _NT, preferred_element_type=F32)

    def a_finish_kv():
        e = lax.broadcasted_iota(jnp.int32, (WIN, WIN), 0)
        d = lax.broadcasted_iota(jnp.int32, (WIN, WIN), 1)
        for w in range(len(WIN_START)):
            _, heads, first, spare = _win_layout(w)
            keep = None
            for j in range(heads):
                lo = first + j * DH
                blk = ((d >= lo) & (d < lo + DH)
                       & (((e >= lo) & (e < lo + DH)) | (e == spare + j)))
                keep = blk if keep is None else keep | blk
            kvz[w] = jnp.where(keep, kv[w], 0.0).astype(BF16)

    def a_apply(c):
        parts = []
        row = lax.broadcasted_iota(jnp.int32, (8, TC), 0)
        for w in range(len(WIN_START)):
            n_r, heads, first, spare = _win_layout(w)
            nd = _mm(kvz[w, :n_r, :n_r], pq[w, :n_r, tok(c)])
            inv = 1.0 / (nd[spare:spare + 8] + 1e-6)
            for g in range(heads * DH // 8):
                j0, j1 = (8 * g) // DH, (8 * g + 7) // DH
                r = jnp.broadcast_to(inv[j0:j0 + 1], (8, TC))
                if j1 != j0:
                    r = jnp.where(row < j1 * DH - 8 * g, r,
                                  jnp.broadcast_to(inv[j1:j1 + 1], (8, TC)))
                parts.append(nd[first + 8 * g:first + 8 * g + 8] * r)
        return jnp.concatenate(parts, axis=0).astype(BF16)

    def b_proj(c, n):
        qt[:, tok(c)] = _mm(wt_r[D:2 * D, :], n) * (DH ** -0.5 * math.log2(math.e))
        k = _mm(wt_r[2 * D:3 * D, :], n)
        for p in range(H // 2):
            kw[p, tok(c), :] = k[p * PW:(p + 1) * PW].T.astype(BF16)
        vt[:, tok(c)] = _mm(wt_r[3 * D:4 * D, :], n)

    def ks(j):
        return slice(j * KC, (j + 1) * KC)

    def locate(t):
        pair = lax.shift_right_logical(t, NQ.bit_length() - 1)
        return pair * PW, (t & (NQ - 1)) * QB, pair

    class Scores:
        def __init__(self, loc, par, s_ref):
            row0, col0, self.pair = loc
            q = qt[pl.ds(pl.multiple_of(row0, 8), PW), pl.ds(pl.multiple_of(col0, QB), QB)]
            row = lax.broadcasted_iota(jnp.int32, q.shape, 0)
            self.q = jnp.where(row >= DH if par else row < DH, q, 0.0).astype(BF16)
            self.s_ref = s_ref
            self.mx = None

        def chunk(self, j):
            s = _mm(kw[self.pair, ks(j), :], self.q)
            self.s_ref[ks(j), :] = s
            cm = jnp.max(s.reshape(KC // 8, 8, QB), axis=0)
            self.mx = cm if self.mx is None else jnp.maximum(self.mx, cm)

    class Weighted:
        def __init__(self, loc, par, s_ref, mx, acc=None):
            self.v0 = pl.multiple_of(loc[0] + 16 * par, 8)
            vrow = lax.broadcasted_iota(jnp.int32, (24, KC), 0)
            self.ones = vrow < 4 if par else vrow >= DH
            self.par, self.s_ref, self.acc = par, s_ref, acc
            self.m = jnp.max(mx, axis=0, keepdims=True)

        def chunk(self, j):
            p = jnp.exp2(self.s_ref[ks(j), :] - self.m).astype(BF16)
            pv = _mm(jnp.where(self.ones, 1.0, vt[pl.ds(self.v0, 24), ks(j)]), p)
            self.acc = pv if self.acc is None else self.acc + pv

        def result(self):
            return self.acc / (self.acc[0:1] if self.par else self.acc[DH:DH + 1])

    def stage(new, tail, head):
        for j in range(NCH):
            if new is not None:
                new.chunk(j)
            if j < LAG:
                if tail is not None:
                    tail.chunk(NCH - LAG + j)
            elif head is not None:
                head.chunk(j - LAG)

    def emit(loc, even, odd):
        o_e, o_o = even.result(), odd.result()
        row = lax.broadcasted_iota(jnp.int32, (8, QB), 0)
        a = pl.multiple_of(loc[0], 8)
        cols = pl.ds(pl.multiple_of(loc[1], QB), QB)
        ot[pl.ds(a, 16), cols] = o_e[0:16]
        ot[pl.ds(a + 16, 8), cols] = jnp.where(row < 4, o_e[16:24], o_o[0:8])
        ot[pl.ds(a + 24, 16), cols] = o_o[8:24]

    def b_attention():
        n_items = (H // 2) * NQ
        assert (n_items - 1) % UNROLL == 0
        first = locate(jnp.int32(0))
        sc_e = Scores(first, 0, s0)
        stage(sc_e, None, None)
        sc_o = Scores(first, 1, s1)
        pv_e = Weighted(first, 0, s0, sc_e.mx)
        stage(sc_o, None, pv_e)

        def item(t, carry):
            mx_e, acc_e, mx_o, cur, nxt = carry
            pv_e = Weighted(cur, 0, s0, mx_e, acc_e)
            pv_o = Weighted(cur, 1, s1, mx_o)
            sc_e = Scores(nxt, 0, s0)
            stage(sc_e, pv_e, pv_o)
            sc_o = Scores(nxt, 1, s1)
            pv_n = Weighted(nxt, 0, s0, sc_e.mx)
            stage(sc_o, pv_o, pv_n)
            emit(cur, pv_e, pv_o)
            return sc_e.mx, pv_n.acc, sc_o.mx, nxt, locate(jnp.minimum(t + 2, n_items - 1))

        def body(i, carry):
            for u in range(UNROLL):
                carry = item(i * UNROLL + u, carry)
            return carry

        mx_e, acc_e, mx_o, last, _ = lax.fori_loop(
            0, (n_items - 1) // UNROLL, body,
            (sc_e.mx, pv_e.acc, sc_o.mx, first, locate(jnp.int32(1))))
        pv_e = Weighted(last, 0, s0, mx_e, acc_e)
        pv_o = Weighted(last, 1, s1, mx_o)
        stage(None, pv_e, pv_o)
        stage(None, pv_o, None)
        emit(last, pv_e, pv_o)

    def chunks(fn):
        def body(c, carry):
            fn(c)
            return carry
        lax.fori_loop(0, NT, body, 0)

    def load_x(c):
        x = xio[tok(c), :].astype(F32).T
        xt[:, tok(c)] = x
        xn[:, tok(c)] = _layernorm(x)

    def first_phase(c):
        batches = ((), (3, 4), (5, 6), (7,), ())
        for j in range(NT):
            @pl.when(c == j)
            def _():
                if j + 2 < NT:
                    x_copy(j + 2).start()
                for i in batches[j + 1]:
                    w_copies[i].start()
                if j + 1 < NT:
                    x_copy(j + 1).wait()
                for i in batches[j]:
                    w_copies[i].wait()
        transpose_weights(wt_r, jnp.where(c == 0, 0, 3 * D),
                          jnp.maximum(c - 1, 0) * (8 * 128), 9 * 128)
        a_proj(c, xn[:, tok(c)])
        load_x(jnp.minimum(c + 1, NT - 1))

    def a_to_b(c):
        x = xt[:, tok(c)] + _mm(wt_r[0:D, :], a_apply(c))
        xt[:, tok(c)] = x
        b_proj(c, _layernorm(x))

    def b_out(c):
        return xt[:, tok(c)] + _mm(wt_r[4 * D:5 * D, :], ot[:, tok(c)].astype(BF16))

    def b_to_a(c):
        x = b_out(c)
        xt[:, tok(c)] = x
        a_proj(c, _layernorm(x))

    def last_phase(c):
        xio[tok(c), :] = b_out(c).T.astype(xio.dtype)
        o_copy(c).start()

    x_copy(0).start()
    w_copies[0].start()
    kv[...] = jnp.zeros(kv.shape, F32)
    x_copy(0).wait()
    w_copies[1].start()
    load_x(0)
    w_copies[0].wait()
    w_copies[2].start()
    transpose_weights(wt_a, 0, 0, D)
    w_copies[1].wait()
    transpose_weights(wt_a, 0, D, D)
    w_copies[2].wait()
    x_copy(1).start()
    transpose_weights(wt_a, 0, 2 * D, D)
    chunks(first_phase)

    def layer_pair(i, carry):
        a_finish_kv()
        chunks(a_to_b)
        b_attention()

        @pl.when(i == 0)
        def _():
            kv[...] = jnp.zeros(kv.shape, F32)
            chunks(b_to_a)
        return carry
    lax.fori_loop(0, 2, layer_pair, 0)

    chunks(last_phase)
    for c in range(NT):
        o_copy(c).wait()


@jax.jit
def pallas_interleave_layers__linear_attn_block__mha_block__prompt_kernel(
    A_x: jax.Array,
    A_wqkv: jax.Array,
    A_wo: jax.Array,
    B_x: jax.Array,
    B_wqkv: jax.Array,
    B_wo: jax.Array,
):
    del B_x
    vmem = pltpu.VMEM
    hbm = pl.BlockSpec(memory_space=pl.ANY)
    nw = len(WIN_START)
    out = pl.pallas_call(
        _kernel,
        out_shape=jax.ShapeDtypeStruct((S, D), A_x.dtype),
        in_specs=[hbm] * 5,
        out_specs=hbm,
        scratch_shapes=[
            vmem((S, D), A_x.dtype),
            vmem((D, 8 * D), A_wqkv.dtype),
            vmem((3 * D, D), BF16), vmem((5 * D, D), BF16),
            vmem((D, S), F32), vmem((D, S), BF16),
            vmem((nw, WIN, S), BF16),
            vmem((nw, WIN, WIN), F32), vmem((nw, WIN, WIN), BF16),
            vmem((D, S), F32), vmem((H // 2, S, PW), BF16),
            vmem((D, S), F32), vmem((D, S), F32),
            vmem((S, QB), F32), vmem((S, QB), F32),
            pltpu.SemaphoreType.DMA((NT,)), pltpu.SemaphoreType.DMA((8,)),
            pltpu.SemaphoreType.DMA((NT,)),
        ],
        compiler_params=pltpu.CompilerParams(vmem_limit_bytes=100 * 1024 * 1024),
        name="interleaved_attn",
    )(A_x.reshape(S, D), A_wqkv, A_wo, B_wqkv, B_wo)
    return out.reshape(A_x.shape)
```

```python
import math

import jax
import jax.numpy as jnp
from jax import lax
import jax.experimental.pallas as pl
import jax.experimental.pallas.tpu as pltpu

S = 2048
D = 640
H = 32
DH = D // H
PW = 2 * DH
WIN = 128
WIN_START = (0, 120, 240, 360, 480, 592)
TC = 512
NT = S // TC
QB = 512
NQ = S // QB
KC = 128
NCH = S // KC
LAG = 3
UNROLL = 3
F32 = jnp.float32
BF16 = jnp.bfloat16

_NT = (((1,), (1,)), ((), ()))


def _mm(a, b):
    return jnp.dot(a, b, preferred_element_type=F32)


def _phi(t):
    return jnp.where(t > 0, t + 1.0, jnp.exp(t)) + 1e-6


def _layernorm(x):
    m = jnp.mean(x, axis=0, keepdims=True)
    xc = x - m
    v = jnp.mean(xc * xc, axis=0, keepdims=True)
    return (xc / jnp.sqrt(v + 1e-5)).astype(BF16)


def _win_layout(w):
    return (48, 2, 8, 0) if w == 5 else (WIN, 6, 0, 120)


def _kernel(x_hbm, waq_hbm, wao_hbm, wbq_hbm, wbo_hbm, o_hbm,
            xio, wst, wt_a, wt_r, xt, xn, pq, kv, kvz, qt, kw, vt, ot, s0, s1,
            x_sem, a_sem, r_sem, o_sem):

    def tok(c):
        return pl.ds(pl.multiple_of(c * TC, TC), TC)

    def x_copy(c):
        return pltpu.make_async_copy(x_hbm.at[tok(c), :], xio.at[tok(c), :], x_sem.at[c])

    def o_copy(c):
        return pltpu.make_async_copy(xio.at[tok(c), :], o_hbm.at[tok(c), :], o_sem.at[c])

    nb = D // 128
    a_copies = [pltpu.make_async_copy(waq_hbm.at[i * 128:(i + 1) * 128, :],
                                      wst.at[i * 128:(i + 1) * 128, :3 * D], a_sem.at[i])
                for i in range(nb)]
    r_src = [wao_hbm] + [wbq_hbm.at[:, j * D:(j + 1) * D] for j in range(3)] + [wbo_hbm]
    r_copies = [pltpu.make_async_copy(src, wst.at[:, (3 + j) * D:(4 + j) * D], r_sem.at[j])
                for j, src in enumerate(r_src)]

    def transposed(w):
        return w.astype(F32).T.astype(BF16)

    def a_proj(c, n):
        q = _phi(_mm(wt_a[0:D, :], n))
        k = _phi(_mm(wt_a[D:2 * D, :], n))
        v = _mm(wt_a[2 * D:3 * D, :], n)
        for w, r0 in enumerate(WIN_START):
            n_r, _, _, spare = _win_layout(w)
            pq[w, :n_r, tok(c)] = q[r0:r0 + n_r].astype(BF16)
            row = lax.broadcasted_iota(jnp.int32, (n_r, TC), 0)
            vw = jnp.where((row >= spare) & (row < spare + 8), 1.0, v[r0:r0 + n_r])
            kv[w, :n_r, :n_r] += lax.dot_general(
                vw.astype(BF16), k[r0:r0 + n_r].astype(BF16), _NT, preferred_element_type=F32)

    def a_finish_kv():
        e = lax.broadcasted_iota(jnp.int32, (WIN, WIN), 0)
        d = lax.broadcasted_iota(jnp.int32, (WIN, WIN), 1)
        for w in range(len(WIN_START)):
            _, heads, first, spare = _win_layout(w)
            keep = None
            for j in range(heads):
                lo = first + j * DH
                blk = ((d >= lo) & (d < lo + DH)
                       & (((e >= lo) & (e < lo + DH)) | (e == spare + j)))
                keep = blk if keep is None else keep | blk
            kvz[w] = jnp.where(keep, kv[w], 0.0).astype(BF16)

    def a_apply(c):
        parts = []
        row = lax.broadcasted_iota(jnp.int32, (8, TC), 0)
        for w in range(len(WIN_START)):
            n_r, heads, first, spare = _win_layout(w)
            nd = _mm(kvz[w, :n_r, :n_r], pq[w, :n_r, tok(c)])
            inv = 1.0 / (nd[spare:spare + 8] + 1e-6)
            for g in range(heads * DH // 8):
                j0, j1 = (8 * g) // DH, (8 * g + 7) // DH
                r = jnp.broadcast_to(inv[j0:j0 + 1], (8, TC))
                if j1 != j0:
                    r = jnp.where(row < j1 * DH - 8 * g, r,
                                  jnp.broadcast_to(inv[j1:j1 + 1], (8, TC)))
                parts.append(nd[first + 8 * g:first + 8 * g + 8] * r)
        return jnp.concatenate(parts, axis=0).astype(BF16)

    def b_proj(c, n):
        qt[:, tok(c)] = _mm(wt_r[D:2 * D, :], n) * (DH ** -0.5 * math.log2(math.e))
        k = _mm(wt_r[2 * D:3 * D, :], n)
        for p in range(H // 2):
            kw[p, tok(c), :] = k[p * PW:(p + 1) * PW].T.astype(BF16)
        vt[:, tok(c)] = _mm(wt_r[3 * D:4 * D, :], n)

    def ks(j):
        return slice(j * KC, (j + 1) * KC)

    def locate(t):
        pair = lax.shift_right_logical(t, NQ.bit_length() - 1)
        return pair * PW, (t & (NQ - 1)) * QB, pair

    class Scores:
        def __init__(self, loc, par, s_ref):
            row0, col0, self.pair = loc
            q = qt[pl.ds(pl.multiple_of(row0, 8), PW), pl.ds(pl.multiple_of(col0, QB), QB)]
            row = lax.broadcasted_iota(jnp.int32, q.shape, 0)
            self.q = jnp.where(row >= DH if par else row < DH, q, 0.0).astype(BF16)
            self.s_ref = s_ref
            self.mx = None

        def chunk(self, j):
            s = _mm(kw[self.pair, ks(j), :], self.q)
            self.s_ref[ks(j), :] = s
            cm = jnp.max(s.reshape(KC // 8, 8, QB), axis=0)
            self.mx = cm if self.mx is None else jnp.maximum(self.mx, cm)

    class Weighted:
        def __init__(self, loc, par, s_ref, mx, acc=None):
            self.v0 = pl.multiple_of(loc[0] + 16 * par, 8)
            vrow = lax.broadcasted_iota(jnp.int32, (24, KC), 0)
            self.ones = vrow < 4 if par else vrow >= DH
            self.par, self.s_ref, self.acc = par, s_ref, acc
            self.m = jnp.max(mx, axis=0, keepdims=True)

        def chunk(self, j):
            p = jnp.exp2(self.s_ref[ks(j), :] - self.m).astype(BF16)
            pv = _mm(jnp.where(self.ones, 1.0, vt[pl.ds(self.v0, 24), ks(j)]), p)
            self.acc = pv if self.acc is None else self.acc + pv

        def result(self):
            return self.acc / (self.acc[0:1] if self.par else self.acc[DH:DH + 1])

    def stage(new, tail, head):
        for j in range(NCH):
            if new is not None:
                new.chunk(j)
            if j < LAG:
                if tail is not None:
                    tail.chunk(NCH - LAG + j)
            elif head is not None:
                head.chunk(j - LAG)

    def emit(loc, even, odd):
        o_e, o_o = even.result(), odd.result()
        row = lax.broadcasted_iota(jnp.int32, (8, QB), 0)
        a = pl.multiple_of(loc[0], 8)
        cols = pl.ds(pl.multiple_of(loc[1], QB), QB)
        ot[pl.ds(a, 16), cols] = o_e[0:16]
        ot[pl.ds(a + 16, 8), cols] = jnp.where(row < 4, o_e[16:24], o_o[0:8])
        ot[pl.ds(a + 24, 16), cols] = o_o[8:24]

    def b_attention():
        n_items = (H // 2) * NQ
        assert (n_items - 1) % UNROLL == 0
        first = locate(jnp.int32(0))
        sc_e = Scores(first, 0, s0)
        stage(sc_e, None, None)
        sc_o = Scores(first, 1, s1)
        pv_e = Weighted(first, 0, s0, sc_e.mx)
        stage(sc_o, None, pv_e)

        def item(t, carry):
            mx_e, acc_e, mx_o, cur, nxt = carry
            pv_e = Weighted(cur, 0, s0, mx_e, acc_e)
            pv_o = Weighted(cur, 1, s1, mx_o)
            sc_e = Scores(nxt, 0, s0)
            stage(sc_e, pv_e, pv_o)
            sc_o = Scores(nxt, 1, s1)
            pv_n = Weighted(nxt, 0, s0, sc_e.mx)
            stage(sc_o, pv_o, pv_n)
            emit(cur, pv_e, pv_o)
            return sc_e.mx, pv_n.acc, sc_o.mx, nxt, locate(jnp.minimum(t + 2, n_items - 1))

        def body(i, carry):
            for u in range(UNROLL):
                carry = item(i * UNROLL + u, carry)
            return carry

        mx_e, acc_e, mx_o, last, _ = lax.fori_loop(
            0, (n_items - 1) // UNROLL, body,
            (sc_e.mx, pv_e.acc, sc_o.mx, first, locate(jnp.int32(1))))
        pv_e = Weighted(last, 0, s0, mx_e, acc_e)
        pv_o = Weighted(last, 1, s1, mx_o)
        stage(None, pv_e, pv_o)
        stage(None, pv_o, None)
        emit(last, pv_e, pv_o)

    def chunks(fn):
        def body(c, carry):
            fn(c)
            return carry
        lax.fori_loop(0, NT, body, 0)

    def load_x(c):
        x = xio[tok(c), :].astype(F32).T
        xt[:, tok(c)] = x
        xn[:, tok(c)] = _layernorm(x)

    def first_phase(c):
        batches = ((), (0, 1), (2, 3), (4,), ())
        for j in range(NT):
            @pl.when(c == j)
            def _():
                if j + 2 < NT:
                    x_copy(j + 2).start()
                for i in batches[j + 1]:
                    r_copies[i].start()
                if j + 1 < NT:
                    x_copy(j + 1).wait()
                for i in batches[j]:
                    r_copies[i].wait()
        dst = pl.multiple_of(jnp.maximum(c - 1, 0) * (8 * 128), 128)
        src = pl.multiple_of(jnp.where(c == 0, 0, 3 * D) + dst, 128)
        wt_r[pl.ds(dst, 9 * 128), :] = transposed(wst[:, pl.ds(src, 9 * 128)])
        a_proj(c, xn[:, tok(c)])
        load_x(jnp.minimum(c + 1, NT - 1))

    def a_to_b(c):
        x = xt[:, tok(c)] + _mm(wt_r[0:D, :], a_apply(c))
        xt[:, tok(c)] = x
        b_proj(c, _layernorm(x))

    def b_out(c):
        return xt[:, tok(c)] + _mm(wt_r[4 * D:5 * D, :], ot[:, tok(c)].astype(BF16))

    def b_to_a(c):
        x = b_out(c)
        xt[:, tok(c)] = x
        a_proj(c, _layernorm(x))

    def last_phase(c):
        xio[tok(c), :] = b_out(c).T.astype(xio.dtype)
        o_copy(c).start()

    x_copy(0).start()
    a_copies[0].start()
    kv[...] = jnp.zeros(kv.shape, F32)
    x_copy(0).wait()
    a_copies[1].start()
    load_x(0)
    for i in range(nb):
        a_copies[i].wait()
        if i + 2 < nb:
            a_copies[i + 2].start()
        elif i + 2 == nb:
            x_copy(1).start()
        wt_a[:, i * 128:(i + 1) * 128] = transposed(wst[i * 128:(i + 1) * 128, :3 * D])
    chunks(first_phase)

    def layer_pair(i, carry):
        a_finish_kv()
        chunks(a_to_b)
        b_attention()

        @pl.when(i == 0)
        def _():
            kv[...] = jnp.zeros(kv.shape, F32)
            chunks(b_to_a)
        return carry
    lax.fori_loop(0, 2, layer_pair, 0)

    chunks(last_phase)
    for c in range(NT):
        o_copy(c).wait()


@jax.jit
def pallas_interleave_layers__linear_attn_block__mha_block__prompt_kernel(
    A_x: jax.Array,
    A_wqkv: jax.Array,
    A_wo: jax.Array,
    B_x: jax.Array,
    B_wqkv: jax.Array,
    B_wo: jax.Array,
):
    del B_x
    vmem = pltpu.VMEM
    hbm = pl.BlockSpec(memory_space=pl.ANY)
    nw = len(WIN_START)
    out = pl.pallas_call(
        _kernel,
        out_shape=jax.ShapeDtypeStruct((S, D), A_x.dtype),
        in_specs=[hbm] * 5,
        out_specs=hbm,
        scratch_shapes=[
            vmem((S, D), A_x.dtype),
            vmem((D, 8 * D), A_wqkv.dtype),
            vmem((3 * D, D), BF16), vmem((5 * D, D), BF16),
            vmem((D, S), F32), vmem((D, S), BF16),
            vmem((nw, WIN, S), BF16),
            vmem((nw, WIN, WIN), F32), vmem((nw, WIN, WIN), BF16),
            vmem((D, S), F32), vmem((H // 2, S, PW), BF16),
            vmem((D, S), F32), vmem((D, S), F32),
            vmem((S, QB), F32), vmem((S, QB), F32),
            pltpu.SemaphoreType.DMA((NT,)), pltpu.SemaphoreType.DMA((D // 128,)),
            pltpu.SemaphoreType.DMA((5,)), pltpu.SemaphoreType.DMA((NT,)),
        ],
        compiler_params=pltpu.CompilerParams(vmem_limit_bytes=100 * 1024 * 1024),
        name="interleaved_attn",
    )(A_x.reshape(S, D), A_wqkv, A_wo, B_wqkv, B_wo)
    return out.reshape(A_x.shape)
```
